```python
import os as _os
_os.environ.setdefault("JAX_PLATFORMS", "cpu")
import jax
import jax.numpy as jnp

def _softmax(x, axis=-1):
    return jax.nn.softmax(x, axis=axis)
def _gelu(x):
    return jax.nn.gelu(x, approximate=True)
def _silu(x):
    return jax.nn.silu(x)
def _sigmoid(x):
    return jax.nn.sigmoid(x)
def _layernorm(x, axis=-1, eps=1e-5):
    m = jnp.mean(x, axis=axis, keepdims=True)
    v = jnp.var(x, axis=axis, keepdims=True)
    return (x - m) / jnp.sqrt(v + eps)
def _scatter_add(tgt, idx, src, axis=0):
    return tgt.at[idx].add(src)
def _segment_sum(src, seg, n):
    return jax.ops.segment_sum(src, seg, n)
class _Rng:
    def __init__(self, key):
        self._k = key
    def _next(self):
        self._k, sub = jax.random.split(self._k)
        return sub
    def normal(self, shape):
        return jax.random.normal(self._next(), shape, dtype=jnp.bfloat16)
    def randint(self, lo, hi, shape):
        return jax.random.randint(self._next(), shape, lo, hi, dtype=jnp.int32)
    def uniform(self, shape, lo=0.0, hi=1.0):
        return jax.random.uniform(self._next(), shape, jnp.bfloat16, lo, hi)
    def permutation(self, n):
        return jax.random.permutation(self._next(), n)


kernel_name = 'concat_heads__gqa_block_cached__gqa_block_cached__near_ridge'

def setup_inputs():
    _rng = _Rng(jax.random.key(int.from_bytes(__import__("os").urandom(4), "little")))
    _w = (lambda a: (lambda t: t.astype(jnp.bfloat16) if jnp.issubdtype(t.dtype, jnp.floating) else t)(jnp.asarray(a)))
    def _A_setup():
        B, Sq, D = 16, 144, 448
        Hq, Hkv, Sk, Dh = 16, 8, 1024, 256
        assert Hq % Hkv == 0, (Hq, Hkv)
        return {
            "x": _w((lambda *s: _rng.normal(s) * 0.8)(B, Sq, D)),
            "k_cache": _w((lambda *s: _rng.normal(s) * 0.8)(B, Hkv, Sk, Dh)),
            "v_cache": _w((lambda *s: _rng.normal(s) * 0.05)(B, Hkv, Sk, Dh)),
            "wq": _w((lambda *s: _rng.normal(s) * 0.8)(D, Hq * Dh) * (D ** -0.5)),
            "wo": _w((lambda *s: _rng.normal(s) * 0.05)(Hq * Dh, D) * ((Hq * Dh) ** -0.5)),
        }
    _A_in = _A_setup()

    def _B_setup():
        B, Sq, D = 16, 144, 448
        Hq, Hkv, Sk, Dh = 16, 8, 1024, 256
        assert Hq % Hkv == 0, (Hq, Hkv)
        return {
            "x": _w((lambda *s: _rng.normal(s) * 0.8)(B, Sq, D)),
            "k_cache": _w((lambda *s: _rng.normal(s) * 0.8)(B, Hkv, Sk, Dh)),
            "v_cache": _w((lambda *s: _rng.normal(s) * 0.05)(B, Hkv, Sk, Dh)),
            "wq": _w((lambda *s: _rng.normal(s) * 0.8)(D, Hq * Dh) * (D ** -0.5)),
            "wo": _w((lambda *s: _rng.normal(s) * 0.05)(Hq * Dh, D) * ((Hq * Dh) ** -0.5)),
        }
    _B_in = _B_setup()

    return {
        "A_x": _A_in["x"],
        "A_k_cache": _A_in["k_cache"],
        "A_v_cache": _A_in["v_cache"],
        "A_wq": _A_in["wq"],
        "A_wo": _A_in["wo"],
        "B_x": _B_in["x"],
        "B_k_cache": _B_in["k_cache"],
        "B_v_cache": _B_in["v_cache"],
        "B_wq": _B_in["wq"],
        "B_wo": _B_in["wo"],
    }

def reference(A_x, A_k_cache, A_v_cache, A_wq, A_wo, B_x, B_k_cache, B_v_cache, B_wq, B_wo):
    def _A_ref(x, k_cache, v_cache, wq, wo):
        B, Sq, D = x.shape
        Hq, Dh = 16, 256
        Hkv = k_cache.shape[1]
        rep = Hq // Hkv
        q = (lambda x, *d: x.transpose(*d))((x @ wq).reshape(B, Sq, Hq, Dh), 0, 2, 1, 3)
        k = jnp.repeat(k_cache, rep, axis=1)
        v = jnp.repeat(v_cache, rep, axis=1)
        scores = jnp.einsum("bhqd,bhkd->bhqk", q, k) * (Dh ** -0.5)
        p = _softmax(scores, axis=-1)
        o = jnp.einsum("bhqk,bhkd->bhqd", p, v)
        return (lambda x, *d: x.transpose(*d))(o, 0, 2, 1, 3).reshape(B, Sq, Hq * Dh) @ wo

    def _B_ref(x, k_cache, v_cache, wq, wo):
        B, Sq, D = x.shape
        Hq, Dh = 16, 256
        Hkv = k_cache.shape[1]
        rep = Hq // Hkv
        q = (lambda x, *d: x.transpose(*d))((x @ wq).reshape(B, Sq, Hq, Dh), 0, 2, 1, 3)
        k = jnp.repeat(k_cache, rep, axis=1)
        v = jnp.repeat(v_cache, rep, axis=1)
        scores = jnp.einsum("bhqd,bhkd->bhqk", q, k) * (Dh ** -0.5)
        p = _softmax(scores, axis=-1)
        o = jnp.einsum("bhqk,bhkd->bhqd", p, v)
        return (lambda x, *d: x.transpose(*d))(o, 0, 2, 1, 3).reshape(B, Sq, Hq * Dh) @ wo

    a = _A_ref(A_x, A_k_cache, A_v_cache, A_wq, A_wo)
    b = _B_ref(B_x, B_k_cache, B_v_cache, B_wq, B_wo)
    return jnp.concatenate([a, b], axis=-1)
```

```python
import numpy as np
import jax
import jax.numpy as jnp
from jax import lax
import jax.experimental.pallas as pl
import jax.experimental.pallas.tpu as pltpu

B, SQ, D = 16, 144, 448
HQ, HKV, SK, DH = 16, 8, 1024, 256
GB = 8
NG = B // GB
GR = GB * SQ
NTILE = GR // 128
HW = (HQ // HKV) * DH
NIT = NG * 2 * HKV
CK = 256
QSCALE = float(DH ** -0.5 * np.log2(np.e))
NT = (((1,), (1,)), ((), ()))
F32 = jnp.float32
BF16 = jnp.bfloat16


def _kernel(xa, ka, va, wqa, woa, xb, kb, vb, wqb, wob, out,
            x_v, wq_v, wo_v, k_v, v_v, q_v, o_v, acc_v, out_v,
            sem_x, sem_wq, sem_wo, sem_k, sem_v, sem_o):
    def decode(t):
        return t >> 4, (t >> 3) & 1, t & 7

    def x_copy(src, br, g):
        return pltpu.make_async_copy(
            src.at[pl.ds(g * GR, GR)], x_v.at[br * NG + g], sem_x.at[br * NG + g])

    def wq_copy(src, br, h):
        return pltpu.make_async_copy(
            src.at[:, pl.ds(h * HW, HW)], wq_v.at[br * HKV + h], sem_wq.at[br * HKV + h])

    def wo_copy(src, br, h):
        return pltpu.make_async_copy(
            src.at[:, pl.ds(h * HW, HW)], wo_v.at[br * HKV + h], sem_wo.at[br * HKV + h])

    def kv_copy(src, dst, sem, slot, g, h, j):
        return pltpu.make_async_copy(
            src.at[g * GB + j, h], dst.at[slot * GB + j], sem.at[slot * GB + j])

    def out_copy(g, i):
        return pltpu.make_async_copy(
            out_v.at[g, pl.ds(i * 128, 128)], out.at[pl.ds(g * GR + i * 128, 128)], sem_o.at[g])

    x0_head = pltpu.make_async_copy(
        xa.at[pl.ds(0, SQ)], x_v.at[0, pl.ds(0, SQ)], sem_x.at[2 * NG])
    x0_tail = pltpu.make_async_copy(
        xa.at[pl.ds(SQ, GR - SQ)], x_v.at[0, pl.ds(SQ, GR - SQ)], sem_x.at[0])

    def start_ab(cond, br, copy_a, copy_b):
        pl.when(jnp.logical_and(cond, br == 0))(lambda: copy_a().start(priority=1))
        pl.when(jnp.logical_and(cond, br == 1))(lambda: copy_b().start(priority=1))

    def qproj(g, br, h, j):
        x = x_v[br * NG + g, pl.ds(j * SQ, SQ), :]
        q = jnp.dot(x, wq_v[br * HKV + h], preferred_element_type=F32)
        q = (q * QSCALE).astype(BF16)
        return jnp.concatenate([q[:, :DH], q[:, DH:]], axis=0)

    def body(t, carry):
        g, br, h = decode(t)
        slot = t & 1
        g1, br1, h1 = decode(jnp.minimum(t + 1, NIT - 1))
        g2, br2, h2 = decode(jnp.minimum(t + 2, NIT - 1))
        more1 = t + 1 < NIT
        more2 = t + 2 < NIT
        rows = pl.ds(pl.multiple_of(br * D, D), D)
        fin_tile = jnp.minimum(t & 15, NTILE - 1)
        fin_rows = pl.ds(pl.multiple_of(fin_tile * 128, 128), 128)

        def oproj(i):
            r = lax.dot_general(wo_v[br * HKV + h], o_v[pl.ds(i * 128, 128), :], NT,
                                preferred_element_type=F32)
            acc_v[g * NTILE + i, rows, :] += r

        def prefetch(j):
            if j == 0:
                start_ab(jnp.logical_and(more1, g1 == 0), br1,
                         lambda: wo_copy(woa, 0, h1), lambda: wo_copy(wob, 1, h1))
            start_ab(more1, br1,
                     lambda: kv_copy(ka, k_v, sem_k, 1 - slot, g1, h1, j),
                     lambda: kv_copy(kb, k_v, sem_k, 1 - slot, g1, h1, j))
            start_ab(more1, br1,
                     lambda: kv_copy(va, v_v, sem_v, 1 - slot, g1, h1, j),
                     lambda: kv_copy(vb, v_v, sem_v, 1 - slot, g1, h1, j))
            if j == GB - 1:
                start_ab(jnp.logical_and(more2, h2 == 0), br2,
                         lambda: x_copy(xa, 0, g2), lambda: x_copy(xb, 1, g2))
                start_ab(jnp.logical_and(more2, g2 == 0), br2,
                         lambda: wq_copy(wqa, 0, h2), lambda: wq_copy(wqb, 1, h2))

        q = q_v[...]
        for j in range(GB):
            kv_copy(ka, k_v, sem_k, slot, g, h, j).wait()
            kr = k_v.at[slot * GB + j]
            vr = v_v.at[slot * GB + j]
            s = jnp.concatenate(
                [lax.dot_general(q, kr[c:c + CK, :], NT, preferred_element_type=F32)
                 for c in range(0, SK, CK)], axis=1)

            if j < 2 * D // 128:
                cols = slice(j * 128, (j + 1) * 128)
                out_v[1 - g, fin_rows, cols] = (
                    acc_v[(1 - g) * NTILE + fin_tile, cols, :].T.astype(BF16))
            if j == GB - 1:
                pl.when(jnp.logical_and(g == 1, (t & 15) < NTILE))(
                    lambda: out_copy(0, fin_tile).start())

            prefetch(j)
            if j + 1 < GB:
                q = qproj(g, br, h, j + 1)
            else:
                pl.when(jnp.logical_and(more1, h1 == 0))(lambda: x_copy(xa, br1, g1).wait())
                pl.when(jnp.logical_and(more1, g1 == 0))(lambda: wq_copy(wqa, br1, h1).wait())
                oproj(j - 1)

            kv_copy(va, v_v, sem_v, slot, g, h, j).wait()
            mx = s[:, :128]
            for c in range(128, SK, 128):
                mx = jnp.maximum(mx, s[:, c:c + 128])
            m = jnp.max(mx, axis=-1, keepdims=True)
            o = None
            ls = None
            for c in range(0, SK, CK):
                ps = [jnp.exp2(s[:, cc:cc + 128] - m) for cc in range(c, c + CK, 128)]
                for p in ps:
                    ls = p if ls is None else ls + p
                pb = jnp.concatenate(ps, axis=1).astype(BF16)
                d = jnp.dot(pb, vr[c:c + CK, :], preferred_element_type=F32)
                o = d if o is None else o + d
            l = jnp.sum(ls, axis=-1, keepdims=True)
            inv = pl.reciprocal(l, approx=True)
            inv = inv * (2.0 - l * inv)
            o = (o * inv).astype(BF16)
            o_v[pl.ds(j * SQ, SQ), :DH] = o[:SQ]
            o_v[pl.ds(j * SQ, SQ), DH:] = o[SQ:]
            if j == 1:
                pl.when(g == 0)(lambda: wo_copy(woa, br, h).wait())
            if 1 <= j < GB - 1:
                oproj(j - 1)
        q_v[...] = qproj(g1, br1, h1, 0)
        oproj(GB - 1)
        oproj(GB)
        return carry

    x0_head.start()
    wq_copy(wqa, 0, 0).start()
    for j in range(GB):
        kv_copy(ka, k_v, sem_k, 0, 0, 0, j).start(priority=0 if j < 2 else 1)
        if j == 0:
            x0_tail.start()
        kv_copy(va, v_v, sem_v, 0, 0, 0, j).start(priority=0 if j < 1 else 1)
        if j == 0:
            wo_copy(woa, 0, 0).start()
    wq_copy(wqa, 0, 1).start(priority=1)
    acc_v[...] = jnp.zeros_like(acc_v)
    x0_head.wait()
    wq_copy(wqa, 0, 0).wait()
    q_v[...] = qproj(0, 0, 0, 0)
    x0_tail.wait()

    lax.fori_loop(0, NIT, body, None)

    g = NG - 1
    for i in range(NTILE):
        out_v[g, pl.ds(i * 128, 128), :] = acc_v[g * NTILE + i].T.astype(BF16)
        out_copy(g, i).start()
    for g in range(NG):
        pltpu.make_async_copy(out_v.at[g], out.at[pl.ds(g * GR, GR)], sem_o.at[g]).wait()


@jax.jit
def pallas_concat_heads__gqa_block_cached__gqa_block_cached__near_ridge_kernel(
    A_x: jax.Array,
    A_k_cache: jax.Array,
    A_v_cache: jax.Array,
    A_wq: jax.Array,
    A_wo: jax.Array,
    B_x: jax.Array,
    B_k_cache: jax.Array,
    B_v_cache: jax.Array,
    B_wq: jax.Array,
    B_wo: jax.Array,
):
    hbm = pl.BlockSpec(memory_space=pltpu.MemorySpace.HBM)
    out = pl.pallas_call(
        _kernel,
        in_specs=[hbm] * 10,
        out_specs=hbm,
        out_shape=jax.ShapeDtypeStruct((B * SQ, 2 * D), BF16),
        scratch_shapes=[
            pltpu.VMEM((2 * NG, GR, D), BF16),
            pltpu.VMEM((2 * HKV, D, HW), BF16),
            pltpu.VMEM((2 * HKV, D, HW), BF16),
            pltpu.VMEM((2 * GB, SK, DH), BF16),
            pltpu.VMEM((2 * GB, SK, DH), BF16),
            pltpu.VMEM((2 * SQ, DH), BF16),
            pltpu.VMEM((GR, HW), BF16),
            pltpu.VMEM((NG * NTILE, 2 * D, 128), F32),
            pltpu.VMEM((NG, GR, 2 * D), BF16),
            pltpu.SemaphoreType.DMA((2 * NG + 1,)),
            pltpu.SemaphoreType.DMA((2 * HKV,)),
            pltpu.SemaphoreType.DMA((2 * HKV,)),
            pltpu.SemaphoreType.DMA((2 * GB,)),
            pltpu.SemaphoreType.DMA((2 * GB,)),
            pltpu.SemaphoreType.DMA((NG,)),
        ],
        compiler_params=pltpu.CompilerParams(
            vmem_limit_bytes=100 * 1024 * 1024,
            disable_bounds_checks=True,
            flags={"XLA_TPU_RESCHEDULE_DMA_DONES": True},
        ),
    )(A_x.reshape(B * SQ, D), A_k_cache, A_v_cache, A_wq, A_wo.T,
      B_x.reshape(B * SQ, D), B_k_cache, B_v_cache, B_wq, B_wo.T)
    return out.reshape(B, SQ, 2 * D)
```

```python
import numpy as np
import jax
import jax.numpy as jnp
from jax import lax
import jax.experimental.pallas as pl
import jax.experimental.pallas.tpu as pltpu

B, SQ, D = 16, 144, 448
HQ, HKV, SK, DH = 16, 8, 1024, 256
GB = 8
NG = B // GB
GR = GB * SQ
NTILE = GR // 128
HW = (HQ // HKV) * DH
NSTEP = NG * 2 * HKV
CK = 256
PW = 512
PO = 2 * D - PW
X0_UNITS = (0, 1, 2, 3, 4, GB)
N_URGENT = 12
QSCALE = float(DH ** -0.5 * np.log2(np.e))
NT = (((1,), (1,)), ((), ()))
F32 = jnp.float32
BF16 = jnp.bfloat16


def _kernel(xa, ka, va, wqa, woa, xb, kb, vb, wqb, wob, out,
            x_v, wq_v, wo_v, k_v, v_v, q_v, o_v, acc_v, out_v,
            sem_x, sem_x0, sem_wq, sem_wo, sem_k, sem_v, sem_o):
    def decode(t):
        return t >> 4, (t >> 3) & 1, t & 7

    def x_copy(src, br, g):
        return pltpu.make_async_copy(
            src.at[pl.ds(g * GR, GR)], x_v.at[br * NG + g], sem_x.at[0])

    def x0_copy(i):
        rows = pl.ds(X0_UNITS[i] * SQ, (X0_UNITS[i + 1] - X0_UNITS[i]) * SQ)
        return pltpu.make_async_copy(xa.at[rows], x_v.at[0, rows], sem_x0.at[i])

    def wq_copy(src, br, h):
        return pltpu.make_async_copy(
            src.at[:, pl.ds(h * HW, HW)], wq_v.at[br * HKV + h], sem_wq.at[h & 1])

    def wo_copy(src, br, h):
        return pltpu.make_async_copy(
            src.at[:, pl.ds(h * HW, HW)], wo_v.at[br * HKV + h], sem_wo.at[h & 1])

    def kv_copy(src, dst, sem, slot, g, h, j):
        return pltpu.make_async_copy(
            src.at[g * GB + j, h], dst.at[slot * GB + j], sem.at[slot * GB + j])

    def out_copy(g, br, i):
        width = PW if br else PO
        return pltpu.make_async_copy(
            out_v.at[g * 2 + br, pl.ds(i * 128, 128), pl.ds(0, width)],
            out.at[pl.ds(g * GR + i * 128, 128), pl.ds(br * PO, width)], sem_o.at[br])

    def start_ab(cond, br, copy_a, copy_b, priority):
        pl.when(jnp.logical_and(cond, br == 0))(lambda: copy_a().start(priority=priority))
        pl.when(jnp.logical_and(cond, br == 1))(lambda: copy_b().start(priority=priority))

    def qproj(g, br, h, j):
        x = x_v[br * NG + g, pl.ds(j * SQ, SQ), :]
        q = jnp.dot(x, wq_v[br * HKV + h], preferred_element_type=F32)
        q = (q * QSCALE).astype(BF16)
        return jnp.concatenate([q[:, :DH], q[:, DH:]], axis=0)

    def body(it, carry):
        g, br, h0 = decode(2 * it)
        acc_rows = pl.ds(pl.multiple_of(br * D, D), D)
        prev = ((it >> 2) + 3) & 3
        gp, bp = prev >> 1, prev & 1
        prev_done = it >= HKV // 2

        def oproj(u, i):
            r = lax.dot_general(wo_v[br * HKV + h0 + u], o_v[pl.ds(i * 128, 128), :], NT,
                                preferred_element_type=F32)
            acc_v[g * NTILE + i, acc_rows, :] += r

        def transpose_block(i, c):
            src = acc_v[gp * NTILE + i, pl.ds(pl.multiple_of(bp * PO + c * 128, 128), 128), :]
            out_v[prev, pl.ds(pl.multiple_of(i * 128, 128), 128), c * 128:(c + 1) * 128] = (
                src.T.astype(BF16))

        def finish_previous_pass(u, j):
            h = h0 + u
            if 1 <= j < 5:
                transpose_block(h, j - 1)
            if j == 4:
                start_ab(prev_done, bp, lambda: out_copy(gp, 0, h), lambda: out_copy(gp, 1, h), 0)
            if 5 <= j < 7:
                transpose_block(NTILE - 1, 2 * u + j - 5)
            if j == 6 and u == 1:
                start_ab(jnp.logical_and(prev_done, h == HKV - 1), bp,
                         lambda: out_copy(gp, 0, NTILE - 1), lambda: out_copy(gp, 1, NTILE - 1), 0)

        q = q_v[...]
        for u in range(2):
            t = 2 * it + u
            h = h0 + u
            g1, br1, h1 = (g, br, h + 1) if u == 0 else decode(jnp.minimum(t + 1, NSTEP - 1))
            g2, br2, h2 = decode(jnp.minimum(t + 2, NSTEP - 2 + u))
            more1 = True if u == 0 else t + 1 < NSTEP
            more2 = t + 2 < NSTEP

            for j in range(GB):
                n = u * GB + j
                kv_copy(ka, k_v, sem_k, u, g, h, j).wait()
                s = jnp.concatenate(
                    [lax.dot_general(q, k_v[n, c:c + CK, :], NT, preferred_element_type=F32)
                     for c in range(0, SK, CK)], axis=1)

                if n + 1 in X0_UNITS[:-1]:
                    pl.when(it == 0)(lambda: x0_copy(X0_UNITS.index(n + 1)).wait())
                if j == 0:
                    start_ab(jnp.logical_and(more1, g1 == 0), br1,
                             lambda: wo_copy(woa, 0, h1), lambda: wo_copy(wob, 1, h1), 1)
                start_ab(more1, br1,
                         lambda: kv_copy(ka, k_v, sem_k, 1 - u, g1, h1, j),
                         lambda: kv_copy(kb, k_v, sem_k, 1 - u, g1, h1, j), 1)
                start_ab(more1, br1,
                         lambda: kv_copy(va, v_v, sem_v, 1 - u, g1, h1, j),
                         lambda: kv_copy(vb, v_v, sem_v, 1 - u, g1, h1, j), 1)
                if j == GB - 1:
                    if u == 0:
                        start_ab(jnp.logical_and(more2, h2 == 0), br2,
                                 lambda: x_copy(xa, 0, g2), lambda: x_copy(xb, 1, g2), 1)
                    start_ab(jnp.logical_and(more2, g2 == 0), br2,
                             lambda: wq_copy(wqa, 0, h2), lambda: wq_copy(wqb, 1, h2), 1)
                    if u == 1:
                        pl.when(jnp.logical_and(more1, h1 == 0))(
                            lambda: x_copy(xa, br1, g1).wait())
                    pl.when(jnp.logical_and(more1, g1 == 0))(
                        lambda: wq_copy(wqa, br1, h1).wait())

                if j + 1 < GB:
                    q = qproj(g, br, h, j + 1)
                elif u == 0:
                    q = qproj(g1, br1, h1, 0)
                else:
                    q_v[...] = qproj(g1, br1, h1, 0)

                kv_copy(va, v_v, sem_v, u, g, h, j).wait()
                mx = s[:, :128]
                for c in range(128, SK, 128):
                    mx = jnp.maximum(mx, s[:, c:c + 128])
                m = jnp.max(mx, axis=-1, keepdims=True)
                o = ls = d = None
                for c in range(0, SK, CK):
                    mc = m
                    if n in (0, 2 * GB - 1) and d is not None:
                        mc = jnp.where(it < 0, d[:, :128], m)
                    ps = [jnp.exp2(s[:, cc:cc + 128] - mc) for cc in range(c, c + CK, 128)]
                    for p in ps:
                        ls = p if ls is None else ls + p
                    d = jnp.dot(jnp.concatenate(ps, axis=1).astype(BF16), v_v[n, c:c + CK, :],
                                preferred_element_type=F32)
                    o = d if o is None else o + d
                finish_previous_pass(u, j)
                l = jnp.sum(ls, axis=-1, keepdims=True)
                inv = pl.reciprocal(l, approx=True)
                inv = inv * (2.0 - l * inv)
                o = (o * inv).astype(BF16)
                o_v[pl.ds(j * SQ, SQ), :DH] = o[:SQ]
                o_v[pl.ds(j * SQ, SQ), DH:] = o[SQ:]

                if j == 1:
                    pl.when(g == 0)(lambda: wo_copy(woa, br, h).wait())
                if n in (GB, GB + 1):
                    oproj(0, n - 1)
                if j >= 1:
                    oproj(u, j - 1)
        oproj(1, NTILE - 2)
        oproj(1, NTILE - 1)
        return carry

    first = [x0_copy(0), wq_copy(wqa, 0, 0)]
    for j in range(GB):
        first.append(kv_copy(ka, k_v, sem_k, 0, 0, 0, j))
        if j + 1 in X0_UNITS[:-1]:
            first.append(x0_copy(X0_UNITS.index(j + 1)))
        first.append(kv_copy(va, v_v, sem_v, 0, 0, 0, j))
        if j == 1:
            first.append(wo_copy(woa, 0, 0))
    first.append(wq_copy(wqa, 0, 1))

    for copy in first[:4]:
        copy.start()

    def zero(i, carry):
        acc_v[i] = jnp.zeros(acc_v.shape[1:], F32)
        return carry

    lax.fori_loop(0, NG * NTILE, zero, None)
    first[0].wait()
    first[1].wait()
    for i, copy in enumerate(first[4:], 4):
        copy.start(priority=0 if i < N_URGENT else 1)
    q_v[...] = qproj(0, 0, 0, 0)

    lax.fori_loop(0, NSTEP // 2, body, None)

    for i in range(NTILE):
        out_v[2 * NG - 1, pl.ds(i * 128, 128), :] = (
            acc_v[(NG - 1) * NTILE + i, PO:, :].T.astype(BF16))
        out_copy(NG - 1, 1, i).start()
    for br, (lo, hi) in enumerate(((0, PO), (PO, 2 * D))):
        part = out.at[:, pl.ds(lo, hi - lo)]
        pltpu.make_async_copy(part, part, sem_o.at[br]).wait()


@jax.jit
def pallas_concat_heads__gqa_block_cached__gqa_block_cached__near_ridge_kernel(
    A_x: jax.Array,
    A_k_cache: jax.Array,
    A_v_cache: jax.Array,
    A_wq: jax.Array,
    A_wo: jax.Array,
    B_x: jax.Array,
    B_k_cache: jax.Array,
    B_v_cache: jax.Array,
    B_wq: jax.Array,
    B_wo: jax.Array,
):
    hbm = pl.BlockSpec(memory_space=pltpu.MemorySpace.HBM)
    out = pl.pallas_call(
        _kernel,
        in_specs=[hbm] * 10,
        out_specs=hbm,
        out_shape=jax.ShapeDtypeStruct((B * SQ, 2 * D), BF16),
        scratch_shapes=[
            pltpu.VMEM((2 * NG, GR, D), BF16),
            pltpu.VMEM((2 * HKV, D, HW), BF16),
            pltpu.VMEM((2 * HKV, D, HW), BF16),
            pltpu.VMEM((2 * GB, SK, DH), BF16),
            pltpu.VMEM((2 * GB, SK, DH), BF16),
            pltpu.VMEM((2 * SQ, DH), BF16),
            pltpu.VMEM((GR, HW), BF16),
            pltpu.VMEM((NG * NTILE, 2 * D, 128), F32),
            pltpu.VMEM((2 * NG, GR, PW), BF16),
            pltpu.SemaphoreType.DMA((1,)),
            pltpu.SemaphoreType.DMA((len(X0_UNITS) - 1,)),
            pltpu.SemaphoreType.DMA((2,)),
            pltpu.SemaphoreType.DMA((2,)),
            pltpu.SemaphoreType.DMA((2 * GB,)),
            pltpu.SemaphoreType.DMA((2 * GB,)),
            pltpu.SemaphoreType.DMA((2,)),
        ],
        compiler_params=pltpu.CompilerParams(
            vmem_limit_bytes=100 * 1024 * 1024,
            flags={"XLA_TPU_RESCHEDULE_DMA_DONES": True},
        ),
    )(A_x.reshape(B * SQ, D), A_k_cache, A_v_cache, A_wq, A_wo.T,
      B_x.reshape(B * SQ, D), B_k_cache, B_v_cache, B_wq, B_wo.T)
    return out.reshape(B, SQ, 2 * D)
```

```python
import numpy as np
import jax
import jax.numpy as jnp
from jax import lax
import jax.experimental.pallas as pl
import jax.experimental.pallas.tpu as pltpu

B, SQ, D = 16, 144, 448
HQ, HKV, SK, DH = 16, 8, 1024, 256
GB = 8
NG = B // GB
GR = GB * SQ
NTILE = GR // 128
HW = (HQ // HKV) * DH
NSTEP = NG * 2 * HKV
CK = 256
PW = 512
PO = 2 * D - PW
X0_UNITS = (0, 1, 2, 3, 4, GB)
N_URGENT = 11
QSCALE = float(DH ** -0.5 * np.log2(np.e))
NT = (((1,), (1,)), ((), ()))
F32 = jnp.float32
BF16 = jnp.bfloat16


def _kernel(xa, ka, va, wqa, woa, xb, kb, vb, wqb, wob, out,
            x_v, wq_v, wo_v, k_v, v_v, q_v, o_v, acc_v, out_v,
            sem_x, sem_x0, sem_wq, sem_wo, sem_k, sem_v, sem_o):
    def decode(t):
        return t >> 4, (t >> 3) & 1, t & 7

    def x_copy(src, br, g):
        return pltpu.make_async_copy(
            src.at[pl.ds(g * GR, GR)], x_v.at[br * NG + g], sem_x.at[0])

    def x0_copy(i):
        rows = pl.ds(X0_UNITS[i] * SQ, (X0_UNITS[i + 1] - X0_UNITS[i]) * SQ)
        return pltpu.make_async_copy(xa.at[rows], x_v.at[0, rows], sem_x0.at[i])

    def wq_copy(src, br, h):
        return pltpu.make_async_copy(
            src.at[:, pl.ds(h * HW, HW)], wq_v.at[br * HKV + h], sem_wq.at[h & 1])

    def wo_copy(src, br, h):
        return pltpu.make_async_copy(
            src.at[:, pl.ds(h * HW, HW)], wo_v.at[br * HKV + h], sem_wo.at[h & 1])

    def kv_copy(src, dst, sem, slot, g, h, j):
        return pltpu.make_async_copy(
            src.at[g * GB + j, h], dst.at[slot * GB + j], sem.at[slot * GB + j])

    def out_copy(g, br, i):
        width = PW if br else PO
        return pltpu.make_async_copy(
            out_v.at[g * 2 + br, pl.ds(i * 128, 128), pl.ds(0, width)],
            out.at[pl.ds(g * GR + i * 128, 128), pl.ds(br * PO, width)], sem_o.at[br])

    def start_ab(cond, br, copy_a, copy_b, priority):
        pl.when(jnp.logical_and(cond, br == 0))(lambda: copy_a().start(priority=priority))
        pl.when(jnp.logical_and(cond, br == 1))(lambda: copy_b().start(priority=priority))

    def qproj(g, br, h, j):
        x = x_v[br * NG + g, pl.ds(j * SQ, SQ), :]
        q = jnp.dot(x, wq_v[br * HKV + h], preferred_element_type=F32)
        q = (q * QSCALE).astype(BF16)
        return jnp.concatenate([q[:, :DH], q[:, DH:]], axis=0)

    def body(it, carry):
        g, br, h0 = decode(2 * it)
        acc_rows = pl.ds(pl.multiple_of(br * D, D), D)
        prev = ((it >> 2) + 3) & 3
        gp, bp = prev >> 1, prev & 1
        prev_done = it >= HKV // 2

        def oproj(u, i):
            r = lax.dot_general(wo_v[br * HKV + h0 + u], o_v[pl.ds(i * 128, 128), :], NT,
                                preferred_element_type=F32)
            acc_v[g * NTILE + i, acc_rows, :] += r

        def transpose_block(i, c):
            src = acc_v[gp * NTILE + i, pl.ds(pl.multiple_of(bp * PO + c * 128, 128), 128), :]
            out_v[prev, pl.ds(pl.multiple_of(i * 128, 128), 128), c * 128:(c + 1) * 128] = (
                src.T.astype(BF16))

        def finish_previous_pass(u, j):
            h = h0 + u
            if 2 <= j < 6:
                transpose_block(h, j - 2)
            if j == 5:
                start_ab(prev_done, bp, lambda: out_copy(gp, 0, h), lambda: out_copy(gp, 1, h), 0)
            if j >= 6:
                transpose_block(NTILE - 1, 2 * u + j - 6)
            if j == 7 and u == 1:
                start_ab(jnp.logical_and(prev_done, h == HKV - 1), bp,
                         lambda: out_copy(gp, 0, NTILE - 1), lambda: out_copy(gp, 1, NTILE - 1), 0)

        q = q_v[...]
        for u in range(2):
            t = 2 * it + u
            h = h0 + u
            g1, br1, h1 = (g, br, h + 1) if u == 0 else decode(jnp.minimum(t + 1, NSTEP - 1))
            g2, br2, h2 = decode(jnp.minimum(t + 2, NSTEP - 2 + u))
            more1 = True if u == 0 else t + 1 < NSTEP
            more2 = t + 2 < NSTEP

            for j in range(GB):
                n = u * GB + j
                kv_copy(ka, k_v, sem_k, u, g, h, j).wait()
                s = jnp.concatenate(
                    [lax.dot_general(q, k_v[n, c:c + CK, :], NT, preferred_element_type=F32)
                     for c in range(0, SK, CK)], axis=1)

                if n + 1 in X0_UNITS[:-1]:
                    pl.when(it == 0)(lambda: x0_copy(X0_UNITS.index(n + 1)).wait())
                if j == 0:
                    start_ab(jnp.logical_and(more1, g1 == 0), br1,
                             lambda: wo_copy(woa, 0, h1), lambda: wo_copy(wob, 1, h1), 1)
                start_ab(more1, br1,
                         lambda: kv_copy(ka, k_v, sem_k, 1 - u, g1, h1, j),
                         lambda: kv_copy(kb, k_v, sem_k, 1 - u, g1, h1, j), 1)
                start_ab(more1, br1,
                         lambda: kv_copy(va, v_v, sem_v, 1 - u, g1, h1, j),
                         lambda: kv_copy(vb, v_v, sem_v, 1 - u, g1, h1, j), 1)
                if j == GB - 1:
                    if u == 0:
                        start_ab(jnp.logical_and(more2, h2 == 0), br2,
                                 lambda: x_copy(xa, 0, g2), lambda: x_copy(xb, 1, g2), 1)
                    start_ab(jnp.logical_and(more2, g2 == 0), br2,
                             lambda: wq_copy(wqa, 0, h2), lambda: wq_copy(wqb, 1, h2), 1)
                    if u == 1:
                        pl.when(jnp.logical_and(more1, h1 == 0))(
                            lambda: x_copy(xa, br1, g1).wait())
                    pl.when(jnp.logical_and(more1, g1 == 0))(
                        lambda: wq_copy(wqa, br1, h1).wait())

                if j + 1 < GB:
                    q = qproj(g, br, h, j + 1)
                elif u == 0:
                    q = qproj(g1, br1, h1, 0)
                else:
                    q_v[...] = qproj(g1, br1, h1, 0)

                kv_copy(va, v_v, sem_v, u, g, h, j).wait()
                mx = s[:, :128]
                for c in range(128, SK, 128):
                    mx = jnp.maximum(mx, s[:, c:c + 128])
                m = jnp.max(mx, axis=-1, keepdims=True)
                o = ls = d = None
                for c in range(0, SK, CK):
                    mc = m
                    if n in (0, 2 * GB - 1) and d is not None:
                        mc = jnp.where(it < 0, d[:, :128], m)
                    ps = [jnp.exp2(s[:, cc:cc + 128] - mc) for cc in range(c, c + CK, 128)]
                    for p in ps:
                        ls = p if ls is None else ls + p
                    d = jnp.dot(jnp.concatenate(ps, axis=1).astype(BF16), v_v[n, c:c + CK, :],
                                preferred_element_type=F32)
                    o = d if o is None else o + d
                finish_previous_pass(u, j)
                l = jnp.sum(ls, axis=-1, keepdims=True)
                inv = pl.reciprocal(l, approx=True)
                inv = inv * (2.0 - l * inv)
                o = (o * inv).astype(BF16)
                o_v[pl.ds(j * SQ, SQ), :DH] = o[:SQ]
                o_v[pl.ds(j * SQ, SQ), DH:] = o[SQ:]

                if j == 1:
                    pl.when(g == 0)(lambda: wo_copy(woa, br, h).wait())
                if n in (GB, GB + 1):
                    oproj(0, n - 1)
                if j >= 1:
                    oproj(u, j - 1)
        oproj(1, NTILE - 2)
        oproj(1, NTILE - 1)
        return carry

    first = [x0_copy(0), wq_copy(wqa, 0, 0)]
    for j in range(GB):
        first.append(kv_copy(ka, k_v, sem_k, 0, 0, 0, j))
        if j + 1 in X0_UNITS[:-1]:
            first.append(x0_copy(X0_UNITS.index(j + 1)))
        first.append(kv_copy(va, v_v, sem_v, 0, 0, 0, j))
        if j == 1:
            first.append(wo_copy(woa, 0, 0))
    first.append(wq_copy(wqa, 0, 1))

    for copy in first[:4]:
        copy.start()

    def zero(i, carry):
        acc_v[i] = jnp.zeros(acc_v.shape[1:], F32)
        return carry

    lax.fori_loop(0, NG * NTILE, zero, None)
    first[0].wait()
    first[1].wait()
    for i, copy in enumerate(first[4:], 4):
        copy.start(priority=0 if i < N_URGENT else 1)
    q_v[...] = qproj(0, 0, 0, 0)

    lax.fori_loop(0, NSTEP // 2, body, None)

    for i in range(NTILE):
        out_v[2 * NG - 1, pl.ds(i * 128, 128), :] = (
            acc_v[(NG - 1) * NTILE + i, PO:, :].T.astype(BF16))
        out_copy(NG - 1, 1, i).start()
    for br, (lo, hi) in enumerate(((0, PO), (PO, 2 * D))):
        part = out.at[:, pl.ds(lo, hi - lo)]
        pltpu.make_async_copy(part, part, sem_o.at[br]).wait()


@jax.jit
def pallas_concat_heads__gqa_block_cached__gqa_block_cached__near_ridge_kernel(
    A_x: jax.Array,
    A_k_cache: jax.Array,
    A_v_cache: jax.Array,
    A_wq: jax.Array,
    A_wo: jax.Array,
    B_x: jax.Array,
    B_k_cache: jax.Array,
    B_v_cache: jax.Array,
    B_wq: jax.Array,
    B_wo: jax.Array,
):
    hbm = pl.BlockSpec(memory_space=pltpu.MemorySpace.HBM)
    out = pl.pallas_call(
        _kernel,
        in_specs=[hbm] * 10,
        out_specs=hbm,
        out_shape=jax.ShapeDtypeStruct((B * SQ, 2 * D), BF16),
        scratch_shapes=[
            pltpu.VMEM((2 * NG, GR, D), BF16),
            pltpu.VMEM((2 * HKV, D, HW), BF16),
            pltpu.VMEM((2 * HKV, D, HW), BF16),
            pltpu.VMEM((2 * GB, SK, DH), BF16),
            pltpu.VMEM((2 * GB, SK, DH), BF16),
            pltpu.VMEM((2 * SQ, DH), BF16),
            pltpu.VMEM((GR, HW), BF16),
            pltpu.VMEM((NG * NTILE, 2 * D, 128), F32),
            pltpu.VMEM((2 * NG, GR, PW), BF16),
            pltpu.SemaphoreType.DMA((1,)),
            pltpu.SemaphoreType.DMA((len(X0_UNITS) - 1,)),
            pltpu.SemaphoreType.DMA((2,)),
            pltpu.SemaphoreType.DMA((2,)),
            pltpu.SemaphoreType.DMA((2 * GB,)),
            pltpu.SemaphoreType.DMA((2 * GB,)),
            pltpu.SemaphoreType.DMA((2,)),
        ],
        compiler_params=pltpu.CompilerParams(
            vmem_limit_bytes=100 * 1024 * 1024,
            flags={"XLA_TPU_RESCHEDULE_DMA_DONES": True},
        ),
    )(A_x.reshape(B * SQ, D), A_k_cache, A_v_cache, A_wq, A_wo.T,
      B_x.reshape(B * SQ, D), B_k_cache, B_v_cache, B_wq, B_wo.T)
    return out.reshape(B, SQ, 2 * D)
```
